```python
import os as _os
_os.environ.setdefault("JAX_PLATFORMS", "cpu")
import jax
import jax.numpy as jnp

def _softmax(x, axis=-1):
    return jax.nn.softmax(x, axis=axis)
def _gelu(x):
    return jax.nn.gelu(x, approximate=True)
def _silu(x):
    return jax.nn.silu(x)
def _sigmoid(x):
    return jax.nn.sigmoid(x)
def _layernorm(x, axis=-1, eps=1e-5):
    m = jnp.mean(x, axis=axis, keepdims=True)
    v = jnp.var(x, axis=axis, keepdims=True)
    return (x - m) / jnp.sqrt(v + eps)
def _scatter_add(tgt, idx, src, axis=0):
    return tgt.at[idx].add(src)
def _segment_sum(src, seg, n):
    return jax.ops.segment_sum(src, seg, n)
class _Rng:
    def __init__(self, key):
        self._k = key
    def _next(self):
        self._k, sub = jax.random.split(self._k)
        return sub
    def normal(self, shape):
        return jax.random.normal(self._next(), shape, dtype=jnp.bfloat16)
    def randint(self, lo, hi, shape):
        return jax.random.randint(self._next(), shape, lo, hi, dtype=jnp.int32)
    def uniform(self, shape, lo=0.0, hi=1.0):
        return jax.random.uniform(self._next(), shape, jnp.bfloat16, lo, hi)
    def permutation(self, n):
        return jax.random.permutation(self._next(), n)


kernel_name = 'standalone__mha_softmax__sampling'

def setup_inputs():
    _rng = _Rng(jax.random.key(int.from_bytes(__import__("os").urandom(4), "little")))
    _w = (lambda a: (lambda t: t.astype(jnp.bfloat16) if jnp.issubdtype(t.dtype, jnp.floating) else t)(jnp.asarray(a)))
    B, H, Sq, Sk, D = 8, 32, 32, 2048, 128
    return {
        "q": _w((lambda *s: _rng.normal(s) * 0.4)(B, H, Sq, D)),
        "k": _w((lambda *s: _rng.normal(s) * 0.4)(B, H, Sk, D)),
        "v": _w((lambda *s: _rng.normal(s) * 0.05)(B, H, Sk, D)),
    }

def reference(q, k, v):
    scale = q.shape[-1] ** -0.5
    scores = jnp.einsum("bhqd,bhkd->bhqk", q, k) * scale
    p = _softmax(scores, axis=-1)
    return jnp.einsum("bhqk,bhkd->bhqd", p, v)
```

```python
import jax
import jax.numpy as jnp
import jax.experimental.pallas as pl
import jax.experimental.pallas.tpu as pltpu

_STREAMS = 8
_LEAD = 2
_CHUNK_ROWS = 128
_SLOTS = 16
_FLUSH_LEAD = 4


def _attend(q, k_ref, v_ref):
    scale = q.shape[-1] ** -0.5
    s = jax.lax.dot_general(
        q, k_ref[...], (((1,), (1,)), ((), ())), preferred_element_type=jnp.float32
    ) * scale
    m = jnp.max(s, axis=-1, keepdims=True)
    p = jnp.exp(s - m)
    l = jnp.sum(p, axis=-1, keepdims=True)
    o = jnp.dot(p.astype(v_ref.dtype), v_ref[...], preferred_element_type=jnp.float32)
    return o / l


def _kernel(q_hbm, k_hbm, v_hbm, o_hbm, q_buf, o_buf, k_buf, v_buf, k_sem, v_sem, q_sem, o_sem):
    regions, per_region, sk, _ = k_hbm.shape
    n_heads = regions * per_region
    n_chunks = sk // _CHUNK_ROWS
    per_step = n_chunks // _STREAMS

    def locate(t):
        if isinstance(t, int):
            return t % regions, t // regions, t % _SLOTS
        return jax.lax.rem(t, regions), jax.lax.div(t, regions), jax.lax.rem(t, _SLOTS)

    def fetch(t, chunk):
        region, index, slot = locate(t)
        row = chunk * _CHUNK_ROWS
        if not isinstance(row, int):
            row = pl.multiple_of(row, _CHUNK_ROWS)
        rows = pl.ds(row, _CHUNK_ROWS)
        for priority, (src, dst, sem) in enumerate(((k_hbm, k_buf, k_sem), (v_hbm, v_buf, v_sem))):
            pltpu.make_async_copy(
                src.at[region, index, rows], dst.at[slot, rows], sem.at[slot]
            ).start(priority=priority)

    def requests(step):
        out = []
        for i in range(per_step):
            chunk = per_step * step + i
            chunk = chunk % n_chunks if isinstance(step, int) else jax.lax.rem(chunk, n_chunks)
            out += [(step + _LEAD + j, chunk) for j in range(1, _STREAMS + 1)]
        return out

    def process(t):
        region, index, slot = locate(t)
        pltpu.make_async_copy(k_buf.at[slot], k_buf.at[slot], k_sem.at[slot]).wait()
        pltpu.make_async_copy(v_buf.at[slot], v_buf.at[slot], v_sem.at[slot]).wait()
        out = _attend(q_buf[region, index], k_buf.at[slot], v_buf.at[slot])
        o_buf[region, index] = out.astype(o_buf.dtype)

    def flush(lo, hi):
        part = pl.ds(lo, hi - lo)
        pltpu.make_async_copy(o_buf.at[:, part], o_hbm.at[:, part], o_sem).start()

    q_copy = pltpu.make_async_copy(q_hbm, q_buf, q_sem)
    q_copy.start()
    for step in range(-(_LEAD + _STREAMS), 0):
        for t, chunk in requests(step):
            if t >= 0:
                fetch(t, chunk)
    q_copy.wait()

    n_steady = n_heads - _LEAD - _STREAMS

    def steady(t, carry):
        process(t)
        for head, chunk in requests(t):
            fetch(head, chunk)
        return carry

    jax.lax.fori_loop(0, n_steady, steady, None)

    for step in range(n_steady, n_heads):
        for t, chunk in requests(step):
            if t < n_heads:
                fetch(t, chunk)

    flush_at = n_heads - _FLUSH_LEAD
    flushed = flush_at // regions

    def drain(t, carry):
        @pl.when(t == flush_at)
        def _():
            flush(0, flushed)

        process(t)
        return carry

    jax.lax.fori_loop(n_steady, n_heads, drain, None)
    flush(flushed, per_region)
    pltpu.make_async_copy(o_buf, o_buf, o_sem).wait()


@jax.jit
def pallas_standalone__mha_softmax__sampling_kernel(
    q: jax.Array,
    k: jax.Array,
    v: jax.Array,
):
    b, h, sq, d = q.shape
    sk = k.shape[2]
    n_heads = b * h
    assert n_heads % _STREAMS == 0 and n_heads >= _LEAD + _STREAMS
    assert sk % (_CHUNK_ROWS * _STREAMS) == 0
    assert _SLOTS > _LEAD + _STREAMS >= _FLUSH_LEAD
    lead = (_STREAMS, n_heads // _STREAMS)

    out = pl.pallas_call(
        _kernel,
        in_specs=[pl.BlockSpec(memory_space=pl.ANY)] * 3,
        out_specs=pl.BlockSpec(memory_space=pl.ANY),
        out_shape=jax.ShapeDtypeStruct(lead + (sq, d), q.dtype),
        scratch_shapes=[
            pltpu.VMEM(lead + (sq, d), q.dtype),
            pltpu.VMEM(lead + (sq, d), q.dtype),
            pltpu.VMEM((_SLOTS, sk, d), k.dtype),
            pltpu.VMEM((_SLOTS, sk, d), v.dtype),
            pltpu.SemaphoreType.DMA((_SLOTS,)),
            pltpu.SemaphoreType.DMA((_SLOTS,)),
            pltpu.SemaphoreType.DMA(()),
            pltpu.SemaphoreType.DMA(()),
        ],
        compiler_params=pltpu.CompilerParams(vmem_limit_bytes=64 * 1024 * 1024),
    )(q.reshape(lead + (sq, d)), k.reshape(lead + (sk, d)), v.reshape(lead + (sk, d)))
    return out.reshape(b, h, sq, d)
```

```python
import jax
import jax.numpy as jnp
import jax.experimental.pallas as pl
import jax.experimental.pallas.tpu as pltpu

_STREAMS = 8
_LEAD = 2
_IN_FLIGHT = _LEAD + _STREAMS
_CHUNK_ROWS = 128
_SLOTS = 16
_FLUSH_LEAD = 4


def _attend(q, k_ref, v_ref):
    scale = q.shape[-1] ** -0.5
    s = jax.lax.dot_general(
        q, k_ref[...], (((1,), (1,)), ((), ())), preferred_element_type=jnp.float32
    ) * scale
    m = jnp.max(s, axis=-1, keepdims=True)
    p = jnp.exp(s - m)
    l = jnp.sum(p, axis=-1, keepdims=True)
    o = jnp.dot(p.astype(v_ref.dtype), v_ref[...], preferred_element_type=jnp.float32)
    return o / l


def _rem(x, n):
    return x % n if isinstance(x, int) else jax.lax.rem(x, n)


def _div(x, n):
    return x // n if isinstance(x, int) else jax.lax.div(x, n)


def _kernel(q_hbm, k_hbm, v_hbm, o_hbm, q_buf, o_buf, kv_buf, kv_sems, io_sem):
    regions, per_region, sk, _ = k_hbm.shape
    n_heads = regions * per_region
    n_chunks = sk // _CHUNK_ROWS
    per_step = n_chunks // _STREAMS

    def fetch(t, chunk):
        row = chunk * _CHUNK_ROWS
        if not isinstance(row, int):
            row = pl.multiple_of(row, _CHUNK_ROWS)
        rows = pl.ds(row, _CHUNK_ROWS)
        for which, src in enumerate((k_hbm, v_hbm)):
            pltpu.make_async_copy(
                src.at[_rem(t, regions), _div(t, regions), rows],
                kv_buf.at[_rem(t, _SLOTS), which, rows],
                kv_sems.at[_rem(t, _IN_FLIGHT)],
            ).start(priority=which)

    def requests(step):
        return [
            (step + _LEAD + j, _rem(per_step * step + i, n_chunks))
            for i in range(per_step)
            for j in range(1, _STREAMS + 1)
        ]

    def process(t):
        region, index = _rem(t, regions), _div(t, regions)
        kv = kv_buf.at[_rem(t, _SLOTS)]
        pltpu.make_async_copy(kv, kv, kv_sems.at[_rem(t, _IN_FLIGHT)]).wait()
        out = _attend(q_buf[region, index], kv.at[0], kv.at[1])
        o_buf[region, index] = out.astype(o_buf.dtype)

    def copy_heads(src, dst, count, queues):
        group = max(_CHUNK_ROWS // src.shape[2], 1)
        for first in range(0, count, group):
            part = pl.ds(first, min(group, count - first))
            for region in range(regions):
                pltpu.make_async_copy(src.at[region, part], dst.at[region, part], io_sem).start(
                    priority=(first // group) % queues
                )

    copy_heads(q_hbm, q_buf, per_region, queues=1)
    for step in range(-_IN_FLIGHT, 0):
        for t, chunk in requests(step):
            if t >= 0:
                fetch(t, chunk)
    pltpu.make_async_copy(q_hbm, q_buf, io_sem).wait()

    n_steady = n_heads - _IN_FLIGHT

    def steady(t, carry):
        process(t)
        for head, chunk in requests(t):
            fetch(head, chunk)
        return carry

    jax.lax.fori_loop(0, n_steady, steady, None)

    rest = [x for step in range(n_steady, n_heads) for x in requests(step) if x[0] < n_heads]
    batches = [rest[i : i + n_chunks] for i in range(0, len(rest), n_chunks)]
    flush_after = n_heads - _FLUSH_LEAD - 1
    flushed = (flush_after + 1) // regions

    def drain(t, carry):
        process(t)
        for i, batch in enumerate(batches):

            @pl.when(t == n_steady + i)
            def _():
                for head, chunk in batch:
                    fetch(head, chunk)

        @pl.when(t == flush_after)
        def _():
            copy_heads(o_buf, o_hbm, flushed, queues=2)

        return carry

    jax.lax.fori_loop(n_steady, n_heads, drain, None)
    last = pl.ds(flushed, per_region - flushed)
    pltpu.make_async_copy(o_buf.at[:, last], o_hbm.at[:, last], io_sem).start()
    pltpu.make_async_copy(o_buf, o_hbm, io_sem).wait()


@jax.jit
def pallas_standalone__mha_softmax__sampling_kernel(
    q: jax.Array,
    k: jax.Array,
    v: jax.Array,
):
    b, h, sq, d = q.shape
    sk = k.shape[2]
    n_heads = b * h
    assert n_heads % _STREAMS == 0 and n_heads >= _IN_FLIGHT
    assert sk % (_CHUNK_ROWS * _STREAMS) == 0
    assert _SLOTS > _IN_FLIGHT > _FLUSH_LEAD > 0
    assert k.dtype == v.dtype
    heads = (_STREAMS, n_heads // _STREAMS)

    out = pl.pallas_call(
        _kernel,
        in_specs=[pl.BlockSpec(memory_space=pl.ANY)] * 3,
        out_specs=pl.BlockSpec(memory_space=pl.ANY),
        out_shape=jax.ShapeDtypeStruct(heads + (sq, d), q.dtype),
        scratch_shapes=[
            pltpu.VMEM(heads + (sq, d), q.dtype),
            pltpu.VMEM(heads + (sq, d), q.dtype),
            pltpu.VMEM((_SLOTS, 2, sk, d), k.dtype),
            pltpu.SemaphoreType.DMA((_IN_FLIGHT,)),
            pltpu.SemaphoreType.DMA(()),
        ],
        compiler_params=pltpu.CompilerParams(vmem_limit_bytes=64 * 1024 * 1024),
    )(q.reshape(heads + (sq, d)), k.reshape(heads + (sk, d)), v.reshape(heads + (sk, d)))
    return out.reshape(b, h, sq, d)
```
